```python
import os as _os
_os.environ.setdefault('JAX_PLATFORMS', 'cpu')
import jax
import jax.numpy as jnp

def _softmax(x, axis=-1):
    return jax.nn.softmax(x, axis=axis)

def _gelu(x):
    return jax.nn.gelu(x, approximate=True)

def _silu(x):
    return jax.nn.silu(x)

def _sigmoid(x):
    return jax.nn.sigmoid(x)

def _layernorm(x, axis=-1, eps=1e-05):
    m = jnp.mean(x, axis=axis, keepdims=True)
    v = jnp.var(x, axis=axis, keepdims=True)
    return (x - m) / jnp.sqrt(v + eps)

def _scatter_add(tgt, idx, src, axis=0):
    return tgt.at[idx].add(src)

def _segment_sum(src, seg, n):
    return jax.ops.segment_sum(src, seg, n)

class _Rng:

    def __init__(self, key):
        self._k = key

    def _next(self):
        self._k, sub = jax.random.split(self._k)
        return sub

    def normal(self, shape):
        return jax.random.normal(self._next(), shape, dtype=jnp.bfloat16)

    def randint(self, lo, hi, shape):
        return jax.random.randint(self._next(), shape, lo, hi, dtype=jnp.int32)

    def uniform(self, shape, lo=0.0, hi=1.0):
        return jax.random.uniform(self._next(), shape, jnp.bfloat16, lo, hi)

    def permutation(self, n):
        return jax.random.permutation(self._next(), n)
kernel_name = 'sequential_preLN__memory_aug_recurrent_mem_tr__swiglu_ffn__prompt'

def setup_inputs():
    _rng = _Rng(jax.random.key(int.from_bytes(__import__("os").urandom(4), "little")))
    _w = lambda a: (lambda t: t.astype(jnp.bfloat16) if jnp.issubdtype(t.dtype, jnp.floating) else t)(jnp.asarray(a))

    def _A_setup():
        B, S, Dm = (1, 2048, 640)
        H, Dh = (32, 192)
        M, seg = (8, 32)
        seg = min(seg, S)
        S = S // seg * seg
        return {'x': _w((lambda *s: _rng.normal(s) * 0.05)(B, S, Dm)), 'mem0': _w((lambda *s: _rng.normal(s) * 0.1)(B, M, Dm)), 'Wq': _w((lambda *s: _rng.normal(s) * 1.6)(Dm, H, Dh) * Dm ** (-0.5)), 'Wk': _w((lambda *s: _rng.normal(s) * 1.6)(Dm, H, Dh) * Dm ** (-0.5)), 'Wv': _w((lambda *s: _rng.normal(s) * 0.1)(Dm, H, Dh) * Dm ** (-0.5)), 'Wo': _w((lambda *s: _rng.normal(s) * 0.1)(H, Dh, Dm) * (H * Dh) ** (-0.5)), 'seg_len': seg}
    _A_in = _A_setup()

    def _B_setup():
        B, S, D, F = (1, 2048, 640, 1536)
        return {'x': _w((lambda *s: _rng.normal(s) * 0.05)(B, S, D)), 'w_gate': _w((lambda *s: _rng.normal(s) * 0.05)(D, F)), 'w_up': _w((lambda *s: _rng.normal(s) * 0.05)(D, F)), 'w_down': _w((lambda *s: _rng.normal(s) * 0.05)(F, D))}
    _B_in = _B_setup()
    return {'A_x': _A_in['x'], 'A_mem0': _A_in['mem0'], 'A_Wq': _A_in['Wq'], 'A_Wk': _A_in['Wk'], 'A_Wv': _A_in['Wv'], 'A_Wo': _A_in['Wo'], 'A_seg_len': _A_in['seg_len'], 'B_x': _B_in['x'], 'B_w_gate': _B_in['w_gate'], 'B_w_up': _B_in['w_up'], 'B_w_down': _B_in['w_down']}

def reference(A_x, A_mem0, A_Wq, A_Wk, A_Wv, A_Wo, A_seg_len, B_x, B_w_gate, B_w_up, B_w_down):

    def _A_ref(x, mem0, Wq, Wk, Wv, Wo, seg_len):
        B, S, Dm = x.shape
        H, Dh = (Wq.shape[1], Wq.shape[2])
        M = mem0.shape[1]
        scale = Dh ** (-0.5)
        n_seg = S // seg_len
        L = M + seg_len
        idx = jnp.arange(L)
        mask = (idx[:, None] < M) | (idx[:, None] >= idx[None, :])
        mem = mem0
        outs = []
        for s in range(n_seg):
            xs = x[:, s * seg_len:(s + 1) * seg_len, :].copy()
            h = jnp.concatenate([mem, xs], axis=1)
            q = jnp.einsum('btd,dhe->bhte', h, Wq)
            k = jnp.einsum('btd,dhe->bhte', h, Wk)
            v = jnp.einsum('btd,dhe->bhte', h, Wv)
            scores = jnp.einsum('bhqe,bhke->bhqk', q, k) * scale
            scores = jnp.where(mask[None, None], scores, -1000000000.0)
            p = _softmax(scores, axis=-1)
            o = jnp.einsum('bhqk,bhke->bhqe', p, v)
            o = jnp.einsum('bhte,hed->btd', o, Wo)
            mem = o[:, :M, :].copy()
            outs.append(o[:, M:, :])
        return jnp.concatenate(outs, axis=1)

    def _B_ref(x, w_gate, w_up, w_down):
        g = _silu(x @ w_gate)
        u = x @ w_up
        return g * u @ w_down
    x = A_x
    h = x + _A_ref(_layernorm(x, axis=-1), A_mem0, A_Wq, A_Wk, A_Wv, A_Wo, A_seg_len)
    h2 = h + _B_ref(_layernorm(h, axis=-1), B_w_gate, B_w_up, B_w_down)
    return h2
```

```python
import functools

import jax
import jax.numpy as jnp
import jax.experimental.pallas as pl
import jax.experimental.pallas.tpu as pltpu

F32 = jnp.float32
BF16 = jnp.bfloat16
I32 = jnp.int32

LN_EPS = 1e-05
LOG2E = 1.4426950408889634
LANES = 128
WAIT_AT = (0, 1, 2, 3, 5, 9)
FLAGS = {}


def _weave(side):
    out, n = "", 0
    for t in range(1, 46):
        out += "q"
        while n < len(side) and (n + 1) * 45 <= t * (len(side) + 1):
            out += side[n]
            n += 1
    return out


_MID_A = "oofoossoofooppoofooofoo"
_MID_B = "oofoossofofooppoofooofoo"
_TAIL = ["ss" + "f" * 14 + "pp" + "o" * 15 + "f" * 4, "pp" + "o" * 15 + "f" * 4]


def _order(first, third, mids, last):
    return [first, _weave("ss"), _weave(third)] + [_weave(m) for m in mids] + _TAIL + ["o" * 15 + "f" * last]


ORDER_A = _order("q" * 45 + "ffff", "sfsffffppfff", [_MID_A] * 12 + [_MID_A.replace("f", "")], 10)
ORDER_B = _order("", "fsfsffffppffff", [_MID_B] * 12 + [_MID_B.replace("f", "")], 0)


def _dot(a, b, contract=0):
    return jax.lax.dot_general(a, b, (((1,), (contract,)), ((), ())), preferred_element_type=F32)


def _layernorm(x):
    m = jnp.mean(x, axis=-1, keepdims=True)
    d = x - m
    v = jnp.mean(d * d, axis=-1, keepdims=True)
    return d * jax.lax.rsqrt(v + LN_EPS)


def _tiles(a):
    return [a[:, i:i + LANES] for i in range(0, a.shape[1], LANES)]


def _mm(lhs, w_tile, n_out, out, init=None):
    for n in range(n_out):
        acc = None if init is None else init[n]
        for k, a in enumerate(lhs):
            d = _dot(a, w_tile(k, n))
            acc = d if acc is None else acc + d
            if k == len(lhs) - 1:
                out[n] = acc
            yield


def _wtile(ref, *lead, k0=0, n0=0):
    packed = ref.dtype == I32
    kr = LANES // 2 if packed else LANES

    def get(k, n):
        w = ref[(*lead, slice((k0 + k) * kr, (k0 + k + 1) * kr), slice((n0 + n) * LANES, (n0 + n + 1) * LANES))]
        return pltpu.bitcast(w, BF16) if packed else w

    return get


def _drain(gen):
    for _ in gen:
        pass


def _kernel(
    x_hbm, mem_hbm, wq_hbm, wk_hbm, wv_hbm, wo_hbm, wg_hbm, wu_hbm, wd_hbm,
    out_hbm,
    x_v, xh_v, mem_v, xpre, xnext, stage, wgu, wd, wqkv, wo, pre, att, out_v,
    sem_in, sem_w, sem_out,
    *, n_seg, seg, n_mem, n_pair, dh,
):
    pw = 2 * dh
    d_model = x_v.shape[2]
    d_ff = wgu.shape[2]
    n_key = n_mem + seg
    n_blk = n_seg // 2
    n_pre = n_seg * n_mem
    nd = d_model // LANES
    c_exp = (dh ** -0.5) * LOG2E
    neg = -1000000000.0 * LOG2E

    def w_copy(p, j):
        src = (wq_hbm, wk_hbm, wv_hbm, wo_hbm)[j]
        rows = pl.ds(pl.multiple_of(p * pw, pw), pw)
        return pltpu.make_async_copy(src.at[rows, :], stage.at[p, j], sem_w.at[p, j])

    def out_copy(blk):
        r = pl.ds(2 * blk, 2)
        return pltpu.make_async_copy(out_v.at[r], out_hbm.at[r], sem_out)

    cp_xh = pltpu.make_async_copy(x_hbm.at[:, 0:n_mem, :], xh_v, sem_in.at[0])
    cp_rest = [
        pltpu.make_async_copy(mem_hbm, mem_v, sem_in.at[1]),
        pltpu.make_async_copy(x_hbm, x_v, sem_in.at[2]),
        pltpu.make_async_copy(wg_hbm, wgu.at[0], sem_in.at[3]),
        pltpu.make_async_copy(wu_hbm, wgu.at[1], sem_in.at[4]),
        pltpu.make_async_copy(wd_hbm, wd, sem_in.at[5]),
    ]

    cp_xh.start()

    @pl.loop(0, n_pair)
    def _(p):
        for j in range(3):
            w_copy(p, j).start()

    @pl.loop(0, n_pair)
    def _(p):
        w_copy(p, 3).start()

    for c in cp_rest:
        c.start()
    cp_xh.wait()
    xpre[...] = _layernorm(xh_v[...].astype(F32).reshape(n_pre, d_model)).astype(BF16)

    for p in range(n_pair):
        if p in WAIT_AT and p > 0:
            for pp in range(p, min([w for w in WAIT_AT if w > p] + [n_pair])):
                for j in range(3):
                    w_copy(pp, j).wait()
        if p == n_pair - 1:
            for pp in range(n_pair):
                w_copy(pp, 3).wait()
            for c in cp_rest:
                c.wait()
        for j in range(3):
            if p == 0:
                w_copy(p, j).wait()
            for n in range(3):
                cols = slice((3 * j + n) * LANES, (3 * j + n + 1) * LANES)
                wt = stage[p, j, n * LANES:(n + 1) * LANES, :]
                wqkv[p, :, cols] = pltpu.bitcast(wt.T, I32)
                for r in range(0, n_pre if p < n_pair - 1 else n_pre // 2, LANES):
                    pre[p, r:r + LANES, cols] = _dot(xpre[r:r + LANES, :], wt, contract=1)

    def pre_rest():
        for r in range(n_pre // 2, n_pre, 64):
            yield
        for r in range(n_pre // 2, n_pre, 64):
            lhs = _tiles(xpre[r:r + 64, :])
            for t in range(9):
                y = [None]
                yield from _mm(lhs, _wtile(wqkv, n_pair - 1, n0=t), 1, y)
                pre[n_pair - 1, r:r + 64, t * LANES:(t + 1) * LANES] = y[0]

    def ffn(blk):
        hr, fi = [], []
        for r in range(0, 2 * seg, 16):
            v = x_v[2 * blk + r // seg, r % seg:r % seg + 16, :].astype(F32) + att[r:r + 16, :]
            hr.append(v)
            fi.append(_layernorm(v).astype(BF16))
            yield
        y = _tiles(jnp.concatenate(hr, axis=0))
        fi = _tiles(jnp.concatenate(fi, axis=0))
        act = []
        for c in range(d_ff // LANES):
            g, u = [None], [None]
            yield from _mm(fi, _wtile(wgu, 0, n0=c), 1, g)
            sg = g[0] * (1.0 / (1.0 + jnp.exp(-g[0])))
            yield from _mm(fi, _wtile(wgu, 1, n0=c), 1, u)
            act.append((sg * u[0]).astype(BF16))
        for c in range(d_ff // LANES):
            yield from _mm([act[c]], _wtile(wd, k0=c), nd, y, init=y)
        out_v[pl.ds(2 * blk, 2)] = jnp.concatenate(y, axis=1).astype(BF16).reshape(2, seg, d_model)

    def step(s, mem, xn, filler, order, first=False):
        lane = jax.lax.broadcasted_iota(I32, (n_key, LANES), 1)
        row = jax.lax.broadcasted_iota(I32, (n_key, LANES), 0)
        is_a = lane < n_key
        is_b = jnp.logical_and(lane >= n_key, lane < 2 * n_key)
        visible = jnp.logical_or(row < n_mem, row >= jnp.where(is_a, lane, lane - n_key))
        lo_half = lane < (dh - LANES)
        pad = jnp.zeros((2 * n_key, LANES - 2 * n_key), F32)

        h = _tiles(jnp.concatenate([mem, xn[n_mem:, :]], axis=0).astype(BF16))
        rp = pl.ds(pl.multiple_of(s * n_mem, n_mem), n_mem)
        acc = [None] * nd
        st_q, st_v, st_p, st_o = {}, {}, {}, {}

        def stack(t):
            t0, t1, t2 = _tiles(t)
            outer = jnp.concatenate([t0, t2], axis=0)
            inner = jnp.concatenate([jnp.where(lo_half, t1, 0.0), jnp.where(lo_half, 0.0, t1)], axis=0)
            return outer.astype(BF16), inner.astype(BF16)

        def proj(p, j, out):
            y = [None] * 3
            yield from _mm(h, _wtile(wqkv, p, n0=3 * j), 3, y)
            y = jnp.concatenate(y, axis=1)
            out.append(jnp.concatenate([y[0:n_mem], pre[p, rp, j * pw:(j + 1) * pw], y[n_mem:]], axis=0))

        def qkv(p):
            r = []
            yield from proj(p, 1, r)
            ko, ki = stack(r[0])
            kt = (ko.T, ki.T)
            yield from proj(p, 0, r)
            st_q[p] = (r[1], *kt)
            yield from proj(p, 2, r)
            st_v[p] = stack(r[2])

        def softmax(p):
            q, ko, ki = st_q.pop(p)
            q0, q1, q2 = _tiles(q)
            so = jnp.concatenate([_dot(jnp.concatenate([q0, q2], axis=0), ko), pad], axis=1)
            yield
            si = jnp.concatenate([_dot(q1, ki), pad[0:n_key]], axis=1)
            t = jnp.where(visible, (jnp.where(is_a, so[0:n_key], so[n_key:]) + si) * c_exp, neg)
            ma = jnp.max(jnp.where(is_a, t, -jnp.inf), axis=1, keepdims=True)
            mb = jnp.max(jnp.where(is_b, t, -jnp.inf), axis=1, keepdims=True)
            e = jnp.exp2(t - jnp.where(is_a, ma, mb))
            ea = jnp.where(is_a, e, 0.0)
            eb = jnp.where(is_b, e, 0.0)
            pa = ea / jnp.sum(ea, axis=1, keepdims=True)
            pb = eb / jnp.sum(eb, axis=1, keepdims=True)
            st_p[p] = (pa[:, 0:2 * n_key], pb[:, 0:2 * n_key])
            yield

        def pv(p):
            pa, pb = st_p.pop(p)
            vo, vi = st_v.pop(p)
            oo = _dot(jnp.concatenate([pa, pb], axis=0), vo)
            yield
            st_o[p] = [oo[0:n_key], _dot(pa + pb, vi), oo[n_key:]]
            yield

        def oproj(p):
            def repack(k, n):
                w = _wtile(stage, p, 3)(k, n)
                wo[p, k * 64:(k + 1) * 64, n * LANES:(n + 1) * LANES] = pltpu.bitcast(w, I32)
                return w

            yield from _mm(st_o.pop(p), repack if first else _wtile(wo, p), nd, acc, init=acc)

        for i in range(n_pair + 3):
            stages = {"f": filler}
            for name, fn, lag in (("q", qkv, 0), ("s", softmax, 1), ("p", pv, 2), ("o", oproj, 3)):
                stages[name] = fn(i - lag) if 0 <= i - lag < n_pair else iter(())
            for name in order[i]:
                next(stages[name], None)
            for name in "spoq":
                _drain(stages[name])
            if i == 6:
                xn_next = _layernorm(x_v[jnp.minimum(s + 1, n_seg - 1)].astype(F32))
        acc = jnp.concatenate(acc, axis=1)
        return acc[0:n_mem], acc[n_mem:], xn_next

    def two_steps(blk, mem, xn, filler, first=False):
        mem, a0, xn = step(2 * blk, mem, xn, filler, ORDER_A, first)
        mem, a1, xn = step(2 * blk + 1, mem, xn, filler, ORDER_B)
        _drain(filler)
        xnext[...] = xn
        att[0:seg, :] = a0
        att[seg:2 * seg, :] = a1
        return mem

    mem = two_steps(0, mem_v[...].astype(F32), _layernorm(x_v[0].astype(F32)), pre_rest(), first=True)

    def body(blk, mem):
        mem = two_steps(blk, mem, xnext[...], ffn(blk - 1))
        out_copy(blk - 1).start()
        return mem

    jax.lax.fori_loop(1, n_blk, body, mem)

    _drain(ffn(n_blk - 1))
    out_copy(n_blk - 1).start()
    pltpu.make_async_copy(out_v, out_hbm, sem_out).wait()


@functools.partial(jax.jit, static_argnames=("A_seg_len",))
def pallas_sequential_preLN__memory_aug_recurrent_mem_tr__swiglu_ffn__prompt_kernel(
    A_x: jax.Array,
    A_mem0: jax.Array,
    A_Wq: jax.Array,
    A_Wk: jax.Array,
    A_Wv: jax.Array,
    A_Wo: jax.Array,
    A_seg_len: int,
    B_x: jax.Array,
    B_w_gate: jax.Array,
    B_w_up: jax.Array,
    B_w_down: jax.Array,
):
    del B_x
    batch, seq, d_model = A_x.shape
    n_head, dh = A_Wq.shape[1], A_Wq.shape[2]
    n_mem = A_mem0.shape[1]
    seg = int(A_seg_len)
    d_ff = B_w_gate.shape[1]
    n_seg = seq // seg
    n_pair = n_head // 2
    pw = 2 * dh
    assert batch == 1 and seq % seg == 0 and n_seg % 32 == 0
    assert pw == 3 * LANES and n_head == 32 and n_mem == 8 and seg % 16 == 0
    assert 2 * (n_mem + seg) <= LANES

    def wt(w):
        return jnp.transpose(w, (1, 2, 0)).reshape(n_head * dh, d_model)

    out = pl.pallas_call(
        functools.partial(_kernel, n_seg=n_seg, seg=seg, n_mem=n_mem, n_pair=n_pair, dh=dh),
        out_shape=jax.ShapeDtypeStruct((n_seg, seg, d_model), BF16),
        in_specs=[pl.BlockSpec(memory_space=pl.ANY)] * 9,
        out_specs=pl.BlockSpec(memory_space=pl.ANY),
        scratch_shapes=[
            pltpu.VMEM((n_seg, seg, d_model), BF16),
            pltpu.VMEM((n_seg, n_mem, d_model), BF16),
            pltpu.VMEM((n_mem, d_model), BF16),
            pltpu.VMEM((n_seg * n_mem, d_model), BF16),
            pltpu.VMEM((seg, d_model), F32),
            pltpu.VMEM((n_pair, 4, pw, d_model), BF16),
            pltpu.VMEM((2, d_model, d_ff), BF16),
            pltpu.VMEM((d_ff, d_model), BF16),
            pltpu.VMEM((n_pair, d_model // 2, 3 * pw), I32),
            pltpu.VMEM((n_pair, pw // 2, d_model), I32),
            pltpu.VMEM((n_pair, n_seg * n_mem, 3 * pw), F32),
            pltpu.VMEM((2 * seg, d_model), F32),
            pltpu.VMEM((n_seg, seg, d_model), BF16),
            pltpu.SemaphoreType.DMA((6,)),
            pltpu.SemaphoreType.DMA((n_pair, 4)),
            pltpu.SemaphoreType.DMA(()),
        ],
        compiler_params=pltpu.CompilerParams(vmem_limit_bytes=124 * 1024 * 1024, flags=FLAGS),
        name="rmt_block",
    )(
        A_x.reshape(n_seg, seg, d_model),
        A_mem0.reshape(n_mem, d_model),
        wt(A_Wq), wt(A_Wk), wt(A_Wv),
        A_Wo.reshape(n_head * dh, d_model),
        B_w_gate, B_w_up, B_w_down,
    )
    return out.reshape(batch, seq, d_model)
```

```python
import functools

import jax
import jax.numpy as jnp
import jax.experimental.pallas as pl
import jax.experimental.pallas.tpu as pltpu

F32 = jnp.float32
BF16 = jnp.bfloat16
I32 = jnp.int32

LN_EPS = 1e-05
LOG2E = 1.4426950408889634
LANES = 128
WAIT_AT = (0, 1, 2, 3, 5, 6, 9, 15, 27, 42)
DIRECT = (3,)


def _weave(side):
    out, n = "", 0
    for t in range(1, 46):
        out += "q"
        while n < len(side) and (n + 1) * 45 <= t * (len(side) + 1):
            out += side[n]
            n += 1
    return out


ORDER_A = (["q" * 45 + "ffff"]
           + [_weave(m) for m in ["fsfs", "ssfffffppffff"]
              + ["oossoofoofppooofooofo", "oossoofoofpfpooooofoo"] * 6 + ["oossoooopopoffooooooo"]]
           + ["ssfffffffffffffppooooooooooooooofff", "ppooooooooofooooooffff", "oooooooooooooooffffffff"])
ORDER_B = ([_weave(m) for m in ["", "ss", "fsfsffffppff"]
            + ["oososoofofofppooofoffooo", "oossooofoopfpooofoofoo"] * 6 + ["oossooooppooooooooo"]]
           + ["fsffsfffffffffffppooooooooooooooffoff", "ppoooooooooooooooffff", "ooooooooooooooo"])


def _dot(a, b, contract=0):
    return jax.lax.dot_general(a, b, (((1,), (contract,)), ((), ())), preferred_element_type=F32)


def _layernorm(x):
    m = jnp.mean(x, axis=-1, keepdims=True)
    d = x - m
    v = jnp.mean(d * d, axis=-1, keepdims=True)
    return d * jax.lax.rsqrt(v + LN_EPS)


def _tiles(a):
    return [a[:, i:i + LANES] for i in range(0, a.shape[1], LANES)]


def _mm(lhs, w_tile, n_out, out, init=None):
    for n in range(n_out):
        acc = None if init is None else init[n]
        for k, a in enumerate(lhs):
            d = _dot(a, w_tile(k, n))
            acc = d if acc is None else acc + d
            if k == len(lhs) - 1:
                out[n] = acc
            yield


def _wtile(ref, *lead, k0=0, n0=0):
    packed = ref.dtype == I32
    kr = LANES // 2 if packed else LANES

    def get(k, n):
        w = ref[(*lead, slice((k0 + k) * kr, (k0 + k + 1) * kr), slice((n0 + n) * LANES, (n0 + n + 1) * LANES))]
        return pltpu.bitcast(w, BF16) if packed else w

    return get


def _drain(gen):
    for _ in gen:
        pass


def _kernel(
    x_hbm, mem_hbm, wq_hbm, wk_hbm, wv_hbm, wo_hbm, wg_hbm, wu_hbm, wd_hbm,
    out_hbm,
    x_v, xh_v, mem_v, xpre, xnext, stage, wgu, wd, wqkv, wo, pre, att, out_v,
    sem_in, sem_w, sem_out,
    *, n_seg, seg, n_mem, n_pair, dh,
):
    pw = 2 * dh
    d_model = x_v.shape[2]
    d_ff = wgu.shape[2]
    n_key = n_mem + seg
    n_blk = n_seg // 2
    n_pre = n_seg * n_mem
    nd = d_model // LANES
    c_exp = (dh ** -0.5) * LOG2E
    neg = -1000000000.0 * LOG2E

    def w_copy(p, j):
        src = (wq_hbm, wk_hbm, wv_hbm, wo_hbm)[j]
        rows = pl.ds(pl.multiple_of(p * pw, pw), pw)
        return pltpu.make_async_copy(src.at[rows, :], stage.at[p, j], sem_w.at[p, j])

    def out_copy(blk):
        r = pl.ds(2 * blk, 2)
        return pltpu.make_async_copy(out_v.at[r], out_hbm.at[r], sem_out.at[blk])

    cp_xh = pltpu.make_async_copy(x_hbm.at[:, 0:n_mem, :], xh_v, sem_in.at[0])
    cp_seq = [
        pltpu.make_async_copy(mem_hbm, mem_v, sem_in.at[1]),
        pltpu.make_async_copy(x_hbm, x_v, sem_in.at[2]),
    ]
    cp_ffn = [
        pltpu.make_async_copy(wg_hbm, wgu.at[0], sem_in.at[3]),
        pltpu.make_async_copy(wu_hbm, wgu.at[1], sem_in.at[4]),
        pltpu.make_async_copy(wd_hbm, wd, sem_in.at[5]),
    ]

    cp_xh.start()

    @pl.loop(0, n_pair)
    def _(p):
        for j in range(3):
            w_copy(p, j).start()

    for c in cp_seq:
        c.start()

    @pl.loop(0, n_pair)
    def _(p):
        w_copy(p, 3).start()

    for c in cp_ffn:
        c.start()
    cp_xh.wait()
    xpre[...] = _layernorm(xh_v[...].astype(F32).reshape(n_pre, d_model)).astype(BF16)

    shared = [t for t in range(9) if t not in DIRECT]
    deferred = [(n_pair - 1, r, t) for r in range(n_pre // 2, n_pre, 64) for t in shared]
    deferred += [(n_pair - 2, n_pre - 64, t) for t in shared[:36 - len(deferred)]]

    for p in range(n_pair):
        for j in range(3):
            c = 3 * p + j
            if c in WAIT_AT:
                for cc in range(c, min([w for w in WAIT_AT if w > c] + [3 * n_pair])):
                    w_copy(cc // 3, cc % 3).wait()
            if c == WAIT_AT[-1]:
                for cp in cp_seq + [w_copy(pp, 3) for pp in range(n_pair)]:
                    cp.wait()
            for n in range(3):
                cols = slice((3 * j + n) * LANES, (3 * j + n + 1) * LANES)
                wt = stage[p, j, n * LANES:(n + 1) * LANES, :]
                wqkv[p, :, cols] = pltpu.bitcast(wt.T, I32)
                if 3 * j + n not in DIRECT:
                    end = min([r for pp, r, t in deferred if (pp, t) == (p, 3 * j + n)] + [n_pre])
                    for r in range(0, end, LANES):
                        rows = slice(r, min(r + LANES, end))
                        pre[p, rows, cols] = _dot(xpre[rows, :], wt, contract=1)

    def pre_rest():
        for _ in range(4):
            yield
        for p, r, t in deferred:
            y = [None]
            yield from _mm(_tiles(xpre[r:r + 64, :]), _wtile(wqkv, p, n0=t), 1, y)
            pre[p, r:r + 64, t * LANES:(t + 1) * LANES] = y[0]

    def ffn(blk):
        hr, fi = [], []
        for r in range(0, 2 * seg, 16):
            v = x_v[2 * blk + r // seg, r % seg:r % seg + 16, :].astype(F32) + att[r:r + 16, :]
            hr.append(v)
            fi.append(_layernorm(v).astype(BF16))
            yield
        y = _tiles(jnp.concatenate(hr, axis=0))
        fi = _tiles(jnp.concatenate(fi, axis=0))
        act = []
        for c in range(d_ff // LANES):
            g, u = [None], [None]
            yield from _mm(fi, _wtile(wgu, 0, n0=c), 1, g)
            sg = g[0] * (1.0 / (1.0 + jnp.exp(-g[0])))
            yield from _mm(fi, _wtile(wgu, 1, n0=c), 1, u)
            act.append((sg * u[0]).astype(BF16))
        for c in range(d_ff // LANES):
            yield from _mm([act[c]], _wtile(wd, k0=c), nd, y, init=y)
        out_v[pl.ds(2 * blk, 2)] = jnp.concatenate(y, axis=1).astype(BF16).reshape(2, seg, d_model)

    def step(s, mem, xn, filler, order, first=False):
        lane = jax.lax.broadcasted_iota(I32, (n_key, LANES), 1)
        row = jax.lax.broadcasted_iota(I32, (n_key, LANES), 0)
        is_a = lane < n_key
        is_b = jnp.logical_and(lane >= n_key, lane < 2 * n_key)
        visible = jnp.logical_or(row < n_mem, row >= jnp.where(is_a, lane, lane - n_key))
        lo_half = lane < (dh - LANES)
        pad = jnp.zeros((2 * n_key, LANES - 2 * n_key), F32)

        h = _tiles(jnp.concatenate([mem, xn[n_mem:, :]], axis=0).astype(BF16))
        h_all = _tiles(jnp.concatenate([mem, xn], axis=0))
        rp = pl.ds(pl.multiple_of(s * n_mem, n_mem), n_mem)
        acc = [None] * nd
        st_q, st_v, st_p, st_o = {}, {}, {}, {}

        def stack(t):
            t0, t1, t2 = _tiles(t)
            outer = jnp.concatenate([t0, t2], axis=0)
            inner = jnp.concatenate([jnp.where(lo_half, t1, 0.0), jnp.where(lo_half, 0.0, t1)], axis=0)
            return outer.astype(BF16), inner.astype(BF16)

        def proj(p, j, out):
            cols = []
            for t in range(3 * j, 3 * j + 3):
                y = [None]
                yield from _mm(h_all if t in DIRECT else h, _wtile(wqkv, p, n0=t), 1, y)
                if t not in DIRECT:
                    y = [y[0][0:n_mem], pre[p, rp, t * LANES:(t + 1) * LANES], y[0][n_mem:]]
                cols.append(jnp.concatenate(y, axis=0))
            out.append(jnp.concatenate(cols, axis=1))

        def qkv(p):
            r = []
            yield from proj(p, 1, r)
            ko, ki = stack(r[0])
            kt = (ko.T, ki.T)
            yield from proj(p, 0, r)
            st_q[p] = (r[1], *kt)
            yield from proj(p, 2, r)
            st_v[p] = stack(r[2])

        def softmax(p):
            q, ko, ki = st_q.pop(p)
            q0, q1, q2 = _tiles(q)
            so = jnp.concatenate([_dot(jnp.concatenate([q0, q2], axis=0), ko), pad], axis=1)
            yield
            si = jnp.concatenate([_dot(q1, ki), pad[0:n_key]], axis=1)
            t = jnp.where(visible, (jnp.where(is_a, so[0:n_key], so[n_key:]) + si) * c_exp, neg)
            ma = jnp.max(jnp.where(is_a, t, -jnp.inf), axis=1, keepdims=True)
            mb = jnp.max(jnp.where(is_b, t, -jnp.inf), axis=1, keepdims=True)
            e = jnp.exp2(t - jnp.where(is_a, ma, mb))
            ea = jnp.where(is_a, e, 0.0)
            eb = jnp.where(is_b, e, 0.0)
            pa = ea / jnp.sum(ea, axis=1, keepdims=True)
            pb = eb / jnp.sum(eb, axis=1, keepdims=True)
            st_p[p] = (pa[:, 0:2 * n_key], pb[:, 0:2 * n_key])
            yield

        def pv(p):
            pa, pb = st_p.pop(p)
            vo, vi = st_v.pop(p)
            oo = _dot(jnp.concatenate([pa, pb], axis=0), vo)
            yield
            st_o[p] = [oo[0:n_key], _dot(pa + pb, vi), oo[n_key:]]
            yield

        def oproj(p):
            def repack(k, n):
                w = _wtile(stage, p, 3)(k, n)
                wo[p, k * 64:(k + 1) * 64, n * LANES:(n + 1) * LANES] = pltpu.bitcast(w, I32)
                return w

            yield from _mm(st_o.pop(p), repack if first else _wtile(wo, p), nd, acc, init=acc)

        for i in range(n_pair + 3):
            stages = {"f": filler}
            for name, fn, lag in (("q", qkv, 0), ("s", softmax, 1), ("p", pv, 2), ("o", oproj, 3)):
                stages[name] = fn(i - lag) if 0 <= i - lag < n_pair else iter(())
            for name in order[i]:
                next(stages[name], None)
            for name in "spoq":
                _drain(stages[name])
            if i == 6:
                xn_next = _layernorm(x_v[jnp.minimum(s + 1, n_seg - 1)].astype(F32))
        acc = jnp.concatenate(acc, axis=1)
        return acc[0:n_mem], acc[n_mem:], xn_next

    def two_steps(blk, mem, xn, filler, first=False):
        mem, a0, xn = step(2 * blk, mem, xn, filler, ORDER_A, first)
        mem, a1, xn = step(2 * blk + 1, mem, xn, filler, ORDER_B)
        _drain(filler)
        xnext[...] = xn
        att[0:seg, :] = a0
        att[seg:2 * seg, :] = a1
        return mem

    mem = two_steps(0, mem_v[...].astype(F32), _layernorm(x_v[0].astype(F32)), pre_rest(), first=True)

    for c in cp_ffn:
        c.wait()

    def body(blk, mem):
        mem = two_steps(blk, mem, xnext[...], ffn(blk - 1))
        out_copy(blk - 1).start()
        return mem

    jax.lax.fori_loop(1, n_blk, body, mem)

    _drain(ffn(n_blk - 1))
    out_copy(n_blk - 1).start()

    @pl.loop(0, n_blk)
    def _(blk):
        out_copy(blk).wait()


@functools.partial(jax.jit, static_argnames=("A_seg_len",))
def pallas_sequential_preLN__memory_aug_recurrent_mem_tr__swiglu_ffn__prompt_kernel(
    A_x: jax.Array,
    A_mem0: jax.Array,
    A_Wq: jax.Array,
    A_Wk: jax.Array,
    A_Wv: jax.Array,
    A_Wo: jax.Array,
    A_seg_len: int,
    B_x: jax.Array,
    B_w_gate: jax.Array,
    B_w_up: jax.Array,
    B_w_down: jax.Array,
):
    del B_x
    batch, seq, d_model = A_x.shape
    n_head, dh = A_Wq.shape[1], A_Wq.shape[2]
    n_mem = A_mem0.shape[1]
    seg = int(A_seg_len)
    d_ff = B_w_gate.shape[1]
    n_seg = seq // seg
    n_pair = n_head // 2
    pw = 2 * dh
    assert batch == 1 and seq % seg == 0 and n_seg % 32 == 0
    assert pw == 3 * LANES and n_head == 32 and n_mem == 8 and seg % 16 == 0
    assert 2 * (n_mem + seg) <= LANES

    def wt(w):
        return jnp.transpose(w, (1, 2, 0)).reshape(n_head * dh, d_model)

    out = pl.pallas_call(
        functools.partial(_kernel, n_seg=n_seg, seg=seg, n_mem=n_mem, n_pair=n_pair, dh=dh),
        out_shape=jax.ShapeDtypeStruct((n_seg, seg, d_model), BF16),
        in_specs=[pl.BlockSpec(memory_space=pl.ANY)] * 9,
        out_specs=pl.BlockSpec(memory_space=pl.ANY),
        scratch_shapes=[
            pltpu.VMEM((n_seg, seg, d_model), BF16),
            pltpu.VMEM((n_seg, n_mem, d_model), BF16),
            pltpu.VMEM((n_mem, d_model), BF16),
            pltpu.VMEM((n_seg * n_mem, d_model), BF16),
            pltpu.VMEM((seg, d_model), F32),
            pltpu.VMEM((n_pair, 4, pw, d_model), BF16),
            pltpu.VMEM((2, d_model, d_ff), BF16),
            pltpu.VMEM((d_ff, d_model), BF16),
            pltpu.VMEM((n_pair, d_model // 2, 3 * pw), I32),
            pltpu.VMEM((n_pair, pw // 2, d_model), I32),
            pltpu.VMEM((n_pair, n_seg * n_mem, 3 * pw), F32),
            pltpu.VMEM((2 * seg, d_model), F32),
            pltpu.VMEM((n_seg, seg, d_model), BF16),
            pltpu.SemaphoreType.DMA((6,)),
            pltpu.SemaphoreType.DMA((n_pair, 4)),
            pltpu.SemaphoreType.DMA((n_seg // 2,)),
        ],
        compiler_params=pltpu.CompilerParams(vmem_limit_bytes=124 * 1024 * 1024),
        name="rmt_block",
    )(
        A_x.reshape(n_seg, seg, d_model),
        A_mem0.reshape(n_mem, d_model),
        wt(A_Wq), wt(A_Wk), wt(A_Wv),
        A_Wo.reshape(n_head * dh, d_model),
        B_w_gate, B_w_up, B_w_down,
    )
    return out.reshape(batch, seq, d_model)
```
